```python
import os as _os
_os.environ.setdefault("JAX_PLATFORMS", "cpu")
import jax
import jax.numpy as jnp

def _softmax(x, axis=-1):
    return jax.nn.softmax(x, axis=axis)
def _gelu(x):
    return jax.nn.gelu(x, approximate=True)
def _silu(x):
    return jax.nn.silu(x)
def _sigmoid(x):
    return jax.nn.sigmoid(x)
def _layernorm(x, axis=-1, eps=1e-5):
    m = jnp.mean(x, axis=axis, keepdims=True)
    v = jnp.var(x, axis=axis, keepdims=True)
    return (x - m) / jnp.sqrt(v + eps)
def _scatter_add(tgt, idx, src, axis=0):
    return tgt.at[idx].add(src)
def _segment_sum(src, seg, n):
    return jax.ops.segment_sum(src, seg, n)
class _Rng:
    def __init__(self, key):
        self._k = key
    def _next(self):
        self._k, sub = jax.random.split(self._k)
        return sub
    def normal(self, shape):
        return jax.random.normal(self._next(), shape, dtype=jnp.bfloat16)
    def randint(self, lo, hi, shape):
        return jax.random.randint(self._next(), shape, lo, hi, dtype=jnp.int32)
    def uniform(self, shape, lo=0.0, hi=1.0):
        return jax.random.uniform(self._next(), shape, jnp.bfloat16, lo, hi)
    def permutation(self, n):
        return jax.random.permutation(self._next(), n)


kernel_name = 'sequential_preLN__sliding_block__dense_activation_gelu__prompt'

def setup_inputs():
    _rng = _Rng(jax.random.key(int.from_bytes(__import__("os").urandom(4), "little")))
    _w = (lambda a: (lambda t: t.astype(jnp.bfloat16) if jnp.issubdtype(t.dtype, jnp.floating) else t)(jnp.asarray(a)))
    def _A_setup():
        B, S, D = 1, 2048, 640
        return {
            "x": _w((lambda *s: _rng.normal(s) * 0.05)(B, S, D)),
            "wqkv": _w((lambda *s: _rng.normal(s) * 0.05)(D, 3 * D)),
            "wo": _w((lambda *s: _rng.normal(s) * 0.05)(D, D)),
        }
    _A_in = _A_setup()

    def _B_setup():
        B, S, D, F = 1, 2048, 640, 1536
        return {
            "x": _w((lambda *s: _rng.normal(s) * 0.05)(B, S, D)),
            "w1": _w((lambda *s: _rng.normal(s) * 0.8)(D, F) * (D ** -0.5)),
            "b1": _w((lambda *s: _rng.normal(s) * 0.8)(F) * 0.01),
            "w2": _w((lambda *s: _rng.normal(s) * 0.8)(F, D) * (F ** -0.5)),
            "b2": _w((lambda *s: _rng.normal(s) * 0.05)(D) * 0.01),
        }
    _B_in = _B_setup()

    return {
        "A_x": _A_in["x"],
        "A_wqkv": _A_in["wqkv"],
        "A_wo": _A_in["wo"],
        "B_x": _B_in["x"],
        "B_w1": _B_in["w1"],
        "B_b1": _B_in["b1"],
        "B_w2": _B_in["w2"],
        "B_b2": _B_in["b2"],
    }

def reference(A_x, A_wqkv, A_wo, B_x, B_w1, B_b1, B_w2, B_b2):
    def _A_ref(x, wqkv, wo):
        B, S, D = x.shape
        H = 32; Dh = D // H; W = 256
        qkv = (lambda x, *d: x.transpose(*d))((x @ wqkv).reshape(B, S, 3, H, Dh), 2, 0, 3, 1, 4)
        q, k, v = qkv[0], qkv[1], qkv[2]
        scores = jnp.einsum("bhqd,bhkd->bhqk", q, k) * (Dh ** -0.5)
        idx = jnp.arange(S)
        mask = (idx[:, None] - idx[None, :] >= 0) & (idx[:, None] - idx[None, :] < W)
        scores = jnp.where(mask[None, None], scores, -1e9)
        p = _softmax(scores, axis=-1)
        o = jnp.einsum("bhqk,bhkd->bhqd", p, v)
        return (lambda x, *d: x.transpose(*d))(o, 0, 2, 1, 3).reshape(B, S, D) @ wo

    def _B_ref(x, w1, b1, w2, b2):
        h = jnp.einsum("bsd,df->bsf", x, w1) + b1
        h = _gelu(h)
        return jnp.einsum("bsf,fd->bsd", h, w2) + b2

    x = A_x
    h = x + _A_ref(_layernorm(x, axis=-1), A_wqkv, A_wo)
    h2 = h + _B_ref(_layernorm(h, axis=-1), B_w1, B_b1, B_w2, B_b2)
    return h2
```

```python
import functools
import math


import jax
import jax.numpy as jnp
from jax import lax
import jax.experimental.pallas as pl
import jax.experimental.pallas.tpu as pltpu

_H = 32
_W = 256
_QB = 128
_T1 = 512
_T2 = 256
_RC = (64,64)
_CM = "head"
_PM = "int"
_FC = 512
_W2 = "k"
_MERGE0 = 1
_NEG = -1e9
_EPS = 1e-5


def _ln(x):
    m = jnp.mean(x, axis=-1, keepdims=True)
    xc = x - m
    v = jnp.mean(xc * xc, axis=-1, keepdims=True)
    return xc * lax.rsqrt(v + _EPS)


def _gelu(x):
    c = math.sqrt(2.0 / math.pi)
    inner = x * (c + (c * 0.044715) * (x * x))
    hx = 0.5 * x
    return hx + hx * jnp.tanh(inner)


def _round_robin(gens):
    gens = list(gens)
    while gens:
        for g in list(gens):
            if next(g, None) is None:
                gens.remove(g)


def _drain(gen):
    for _ in gen:
        pass


def _spread(main, n_main, side, n_side, lead=0):
    done = 0
    for i in range(n_main):
        next(main, None)
        want = min(n_side, max(0, -(-(i + 1 - lead) * n_side // (n_main - lead))))
        while done < want:
            next(side, None)
            done += 1
    _drain(main)
    _drain(side)


def _kernel(x_h, wqkv_h, wo_h, w1_h, b1_h, w2_h, b2_h, o_h,
            x_s, wqkv_s, wo_s, w1_s, b1_s, w2_s, b2_s, out_s,
            k_s, vt_s, qt_s, ot_s, s_s, p_s, xn_s, att_s, hres_s, hn_s, g_s,
            isem, osem, *, S, D, F, Dh):
    f32, bf16, i32 = jnp.float32, jnp.bfloat16, jnp.int32
    T1, T2 = _T1, _T2
    N1, N2 = S // T1, S // T2
    NG = _H // 4

    x_cp = [pltpu.make_async_copy(x_h.at[pl.ds(i * T1, T1)], x_s.at[pl.ds(i * T1, T1)], isem.at[i])
            for i in range(N1)]
    w_cp = [pltpu.make_async_copy(wqkv_h.at[:, pl.ds(j * D, D)], wqkv_s.at[j], isem.at[N1 + j])
            for j in range(3)]
    r_cp = [pltpu.make_async_copy(a, b, isem.at[N1 + 3 + j]) for j, (a, b) in enumerate(
        [(wo_h, wo_s), (w1_h, w1_s), (b1_h, b1_s), (w2_h, w2_s), (b2_h, b2_s)])]

    def o_cp(i):
        rows = pl.ds(pl.multiple_of(i * T2, T2), T2)
        return pltpu.make_async_copy(out_s.at[rows], o_h.at[rows], osem.at[i])

    x_cp[0].start()
    w_cp[2].start()
    k_s[0:_W // 2, :] = jnp.zeros((_W // 2, k_s.shape[1]), i32)
    vt_s[0:_W // _QB] = jnp.zeros((_W // _QB, D // 2, _QB), i32)

    qscale = (Dh ** -0.5) * math.log2(math.e)

    def ln1(i):
        xn_s[i % 2] = _ln(x_s[i * T1:(i + 1) * T1, :].astype(f32)).astype(bf16)

    def qkv(i):
        def proj(j):
            return jnp.dot(xn_s[i % 2], wqkv_s[j], preferred_element_type=f32)

        def put_t(ref, b0, val):
            for b in range(T1 // _QB):
                ref[b0 + b] = pltpu.bitcast(val[b * _QB:(b + 1) * _QB].astype(bf16).T, i32)

        if i == 0:
            w_cp[2].wait()
            w_cp[0].start()
            w_cp[1].start()
        put_t(vt_s, (_W + i * T1) // _QB, proj(2))
        yield True
        if i == 0:
            w_cp[0].wait()
            w_cp[1].wait()
            for c in x_cp[1:2]:
                c.start()
        put_t(qt_s, i * T1 // _QB, proj(0) * qscale)
        yield True
        if i == 0:
            for c in x_cp[2:] + r_cp:
                c.start()
        if i + 1 < N1:
            x_cp[i + 1].wait()
            ln1(i + 1)
        ki = pltpu.bitcast(proj(1).astype(bf16), i32)
        lane = lax.broadcasted_iota(i32, (T1 // 2, 128), 1)
        r0 = (_W + i * T1) // 2
        for g in range(NG):
            lo = 4 * Dh * g
            m = lo // 128
            kt = ki[:, 128 * m:128 * (m + 1)]
            if (lo + 4 * Dh - 1) // 128 != m:
                kt = jnp.where(lane >= 64, kt, ki[:, 128 * (m + 1):128 * (m + 2)])
            k_s[r0:r0 + T1 // 2, 128 * g:128 * (g + 1)] = kt
        yield True

    def rowmask(n, lo, hi):
        r = 2 * lax.broadcasted_iota(i32, (n // 2, _QB), 0)
        return (jnp.where((r >= lo) & (r < hi), 0xFFFF, 0)
                | jnp.where((r + 1 >= lo) & (r + 1 < hi), -65536, 0))

    def attention(blk):
        static = isinstance(blk, int)
        dji = lax.broadcasted_iota(i32, (8, _QB), 1) - lax.broadcasted_iota(i32, (8, _QB), 0)
        jj2 = 2 * lax.broadcasted_iota(i32, (_QB // 2, _QB), 0)
        ii2 = lax.broadcasted_iota(i32, (_QB // 2, _QB), 1)
        lowm = jnp.where(jj2 <= ii2, 0xFFFF, 0) | jnp.where(jj2 + 1 <= ii2, -65536, 0)
        r8 = lax.broadcasted_iota(i32, (8, _QB), 0)
        zeros = lambda n: jnp.zeros((n // 2, _QB), i32)
        masks = {off: rowmask(32, off, off + Dh) for off in (0, 4, 8, 12)}
        ones_bits = 0x3F803F80
        state = {}
        qblk0 = blk * (T2 // _QB)
        krow0 = blk * (T2 // 2) if static else pl.multiple_of(blk * (T2 // 2), T2 // 2)

        def stage_a(n, qb, g):
            buf = n % 2
            no0 = static and qblk0 + qb < 2
            no1 = static and qblk0 + qb < 1
            qms = []
            for h in range(4 * g, 4 * g + 4):
                r0 = Dh * h
                a = (r0 // 16) * 16
                q2 = qt_s[qblk0 + qb, a // 2:a // 2 + 16, :] & masks[r0 - a]
                p = a % 128
                if p + 32 <= 128:
                    parts = ([zeros(p)] if p else []) + [q2] + ([zeros(96 - p)] if p < 96 else [])
                else:
                    parts = [q2[8:16], zeros(96), q2[0:8]]
                qms.append(jnp.concatenate(parts, axis=0))
            qm = pltpu.bitcast(jnp.concatenate(qms, axis=1), bf16)
            mx = None
            kl = slice(128 * g, 128 * (g + 1))
            offs = [256] + ([] if no0 else [0]) + ([] if no1 else [128])
            neg = jnp.full((8, 4 * _QB), _NEG, f32)
            r = 0
            for rc in _RC:
                rows = []
                for rr in range(r, r + rc, 16):
                    rows += [k_s[pl.ds(krow0 + (qb * _QB + o + rr) // 2, 8), kl] for o in offs]
                s = jnp.dot(pltpu.bitcast(jnp.concatenate(rows, axis=0), bf16), qm, preferred_element_type=f32)
                for i, rr in enumerate(range(r, r + rc, 16)):
                    for e in (0, 8):
                        part = {o: s[16 * (len(offs) * i + t) + e:16 * (len(offs) * i + t) + e + 8]
                                for t, o in enumerate(offs)}
                        s2, s0, s1 = part[256], part.get(0, neg), part.get(128, neg)
                        low = dji >= rr + e
                        sm = jnp.concatenate(
                            [jnp.where(low, s2[:, 128 * u:128 * (u + 1)], s0[:, 128 * u:128 * (u + 1)])
                             for u in range(4)], axis=1)
                        s_s[buf, rr + e:rr + e + 8, :] = sm
                        s_s[buf, 128 + rr + e:128 + rr + e + 8, :] = s1
                        t = jnp.maximum(sm, s1)
                        mx = t if mx is None else jnp.maximum(mx, t)
                r += rc
                yield True
            state[n] = jnp.broadcast_to(jnp.max(mx, axis=0, keepdims=True), (8, 4 * _QB))

        def stage_b(n, qb, g):
            buf = n % 2
            mx = state.pop(n)
            mx = jnp.concatenate([mx, mx], axis=0)
            r = 0
            for rc in _RC:
                for rr in range(r, r + rc, 16):
                    for o in (0, 128):
                        p = jnp.exp2(s_s[buf, o + rr:o + rr + 16, :] - mx).astype(bf16)
                        p_s[buf, (o + rr) // 2:(o + rr) // 2 + 8, :] = pltpu.bitcast(p, i32)
                r += rc
                yield True

        def stage_c(n, qb, g):
            buf = n % 2

            def lhs(h, t):
                a = (Dh * h // 16) * 16
                off = Dh * h - a
                vt = vt_s[qblk0 + qb + t, a // 2:a // 2 + 16, :]
                w = 1 if off == 0 else 0
                mk = masks[off][8 * w:8 * w + 8]
                vm = (vt[8 * w:8 * w + 8] & mk) | (ones_bits & ~mk)
                return jnp.concatenate([vt[0:8], vm] if w else [vm, vt[8:16]], axis=0)

            def rhs(u, t):
                cs = slice(128 * u, 128 * (u + 1))
                if t == 1:
                    return p_s[buf, 64:128, cs]
                return p_s[buf, 0:64, cs] & (lowm if t == 2 else ~lowm)

            acc = [None] * 4
            if _CM == "head":
                for u in range(4):
                    a_ = jnp.concatenate([lhs(4 * g + u, t) for t in range(3)], axis=1)
                    b_ = jnp.concatenate([rhs(u, t) for t in range(3)], axis=0)
                    acc[u] = jnp.dot(pltpu.bitcast(a_, bf16), pltpu.bitcast(b_, bf16), preferred_element_type=f32)
                    if u < 3:
                        yield True
            else:
                for t in range(3):
                    for u in range(4):
                        o = jnp.dot(pltpu.bitcast(lhs(4 * g + u, t), bf16), pltpu.bitcast(rhs(u, t), bf16),
                                    preferred_element_type=f32)
                        acc[u] = o if t == 0 else acc[u] + o
                    if t < 2:
                        yield True
            outs = []
            for u in range(4):
                r0 = Dh * (4 * g + u)
                a = (r0 // 16) * 16
                l = acc[u][31:32] if r0 == a else acc[u][0:1]
                b = (r0 // 8) * 8 - a
                outs.append(acc[u][b:b + 24] * (1.0 / l))
            for w in (0, 2):
                mid = jnp.where(r8 < 4, outs[w][16:24], outs[w + 1][0:8])
                ot_s[qb, 80 * g + 20 * w:80 * g + 20 * w + 40, :] = jnp.concatenate(
                    [outs[w][0:16], mid, outs[w + 1][8:24]], axis=0)
            yield True

        units = [(qb, g) for qb in range(T2 // _QB) for g in range(NG)]
        nu = len(units)
        for n in range(nu + 2):
            gens = []
            if n < nu:
                gens.append(stage_a(n, *units[n]))
            if 0 <= n - 1 < nu:
                gens.append(stage_b(n - 1, *units[n - 1]))
            if 0 <= n - 2 < nu:
                gens.append(stage_c(n - 2, *units[n - 2]))
            _round_robin(gens)
            yield True

    n_att = (T2 // _QB) * NG + 2

    def ffn(blk):
        rows = pl.ds(blk * T2 if isinstance(blk, int) else pl.multiple_of(blk * T2, T2), T2)
        for b in range(T2 // _QB):
            att_s[b * _QB:(b + 1) * _QB, :] = ot_s[b].astype(bf16).T
        yield True
        hres_s[...] = x_s[rows, :].astype(f32) + jnp.dot(att_s[...], wo_s[...], preferred_element_type=f32)
        yield True
        hn_s[...] = _ln(hres_s[...]).astype(bf16)
        yield True
        b1 = b1_s[...].astype(f32).reshape(1, F)
        for c in range(0, F, _FC):
            hmid = jnp.dot(hn_s[...], w1_s[:, c:c + _FC], preferred_element_type=f32) + b1[:, c:c + _FC]
            g_s[:, c:c + _FC] = _gelu(hmid).astype(bf16)
            yield True
        b2 = b2_s[...].astype(f32).reshape(1, D)
        if _W2 == "k":
            y = hres_s[...] + b2
            for c in range(0, F, 512):
                y = y + jnp.dot(g_s[:, c:c + 512], w2_s[c:c + 512, :], preferred_element_type=f32)
                if c + 512 < F:
                    yield True
            out_s[rows, :] = y.astype(out_s.dtype)
        elif _W2 == "n":
            for c in range(0, D, 128):
                y = jnp.dot(g_s[...], w2_s[:, c:c + 128], preferred_element_type=f32)
                out_s[rows, c:c + 128] = (hres_s[:, c:c + 128] + b2[:, c:c + 128] + y).astype(out_s.dtype)
                if c + 128 < D:
                    yield True
        else:
            y = jnp.dot(g_s[...], w2_s[...], preferred_element_type=f32)
            out_s[rows, :] = (hres_s[...] + b2 + y).astype(out_s.dtype)
        o_cp(blk).start()
        yield True

    n_ffn = 3 + F // _FC + {"k": F // 512, "n": D // 128, "all": 1}[_W2]

    x_cp[0].wait()
    ln1(0)
    for i in range(N1 - 1):
        _drain(qkv(i))
    if _MERGE0:
        _spread(attention(0), n_att, qkv(N1 - 1), 3, lead=1)
    else:
        _drain(qkv(N1 - 1))
        _drain(attention(0))
    for c in r_cp:
        c.wait()

    def body(i, carry):
        _spread(attention(i), n_att, ffn(i - 1), n_ffn)
        return carry

    lax.fori_loop(1, N2, body, 0)
    _drain(ffn(N2 - 1))
    for i in range(N2):
        o_cp(i).wait()


@jax.jit
def pallas_sequential_preLN__sliding_block__dense_activation_gelu__prompt_kernel(
    A_x, A_wqkv, A_wo, B_x, B_w1, B_b1, B_w2, B_b2,
):
    B, S, D = A_x.shape
    F = B_w1.shape[1]
    Dh = D // _H
    bf16, f32, i32 = jnp.bfloat16, jnp.float32, jnp.int32
    V = pltpu.VMEM
    out = pl.pallas_call(
        functools.partial(_kernel, S=S, D=D, F=F, Dh=Dh),
        in_specs=[pl.BlockSpec(memory_space=pl.ANY)] * 7,
        out_specs=pl.BlockSpec(memory_space=pl.ANY),
        out_shape=jax.ShapeDtypeStruct((S, D), A_x.dtype),
        scratch_shapes=[
            V((S, D), bf16), V((3, D, D), bf16), V((D, D), bf16), V((D, F), bf16), V((F,), bf16),
            V((F, D), bf16), V((D,), bf16), V((S, D), bf16),
            V(((_W + S) // 2, 128 * _H // 4), i32),
            V(((_W + S) // _QB, D // 2, _QB), i32),
            V((S // _QB, D // 2, _QB), i32),
            V((_T2 // _QB, D, _QB), f32),
            V((2, 256, 512), f32),
            V((2, 128, 512), i32),
            V((2, _T1, D), bf16), V((_T2, D), bf16), V((_T2, D), f32), V((_T2, D), bf16), V((_T2, F), bf16),
            pltpu.SemaphoreType.DMA((S // _T1 + 8,)),
            pltpu.SemaphoreType.DMA((S // _T2,)),
        ],
        compiler_params=pltpu.CompilerParams(vmem_limit_bytes=100 * 2**20),
    )(A_x.reshape(S, D), A_wqkv, A_wo, B_w1, B_b1, B_w2, B_b2)
    return out.reshape(B, S, D)
```

```python
import functools
import math

import jax
import jax.numpy as jnp
from jax import lax
import jax.experimental.pallas as pl
import jax.experimental.pallas.tpu as pltpu

_H = 32
_W = 256
_QB = 128
_T1 = 512
_T2 = 256
_EPS = 1e-5
_V_HEAD = 256
_LAST = 64
_F_CUT = 1024
_PIECES = [(b, r) for b in range(4) for r in (0, 16)]
_CHUNKS = (_PIECES[:6], _PIECES[6:])
_ORDER = "affafafafafafaaaafaaaaaaf"


def _layernorm(x):
    xc = x - jnp.mean(x, axis=-1, keepdims=True)
    var = jnp.mean(xc * xc, axis=-1, keepdims=True)
    return xc * lax.rsqrt(var + _EPS)


def _gelu_x2(x):
    c = math.sqrt(2.0 / math.pi)
    return x + x * jnp.tanh(x * (c + (c * 0.044715) * (x * x)))


def _dot(a, b):
    return jnp.dot(a, b, preferred_element_type=jnp.float32)


def _aligned(i, n):
    return i if isinstance(i, int) else pl.multiple_of(i, n)


def _interleave(gens):
    gens = list(gens)
    while gens:
        gens = [g for g in gens if next(g, False)]


def _trace_in_order(order, a, f):
    for piece in order:
        next(a if piece == "a" else f)
    _interleave([a])
    _interleave([f])


def _kernel(x_h, wqkv_h, wo_h, w1_h, b1_h, w2_h, b2_h, o_h,
            x_s, wqkv_s, wo_s, w1_s, b1_s, w2_s, b2_s, out_s,
            xn_s, k_s, kprev_s, vt_s, qt_s, s0_s, s1_s, ot_s, att_s, h_s, hn_s, g_s,
            in_sem, out_sem, *, S, D, F, Dh):
    f32, bf16, i32 = jnp.float32, jnp.bfloat16, jnp.int32
    T1, T2, QB = _T1, _T2, _QB
    N1, N2, NG = S // T1, S // T2, _H // 4

    def rows_of_x(a, n):
        return x_h.at[pl.ds(a, n)], x_s.at[pl.ds(a, n)]

    def cols_of_wqkv(j, a, n):
        return wqkv_h.at[:, pl.ds(j * D + a, n)], wqkv_s.at[j, :, pl.ds(a, n)]

    pairs = dict(x0=rows_of_x(0, T1),
                 wv0=cols_of_wqkv(2, 0, _V_HEAD), wv1=cols_of_wqkv(2, _V_HEAD, D - _V_HEAD),
                 wk=cols_of_wqkv(1, 0, D), wq=cols_of_wqkv(0, 0, D),
                 x1=rows_of_x(T1, T1), x2=rows_of_x(2 * T1, S - 2 * T1),
                 wo=(wo_h, wo_s), w1=(w1_h, w1_s), b1=(b1_h, b1_s), w2=(w2_h, w2_s), b2=(b2_h, b2_s))
    loads = {name: pltpu.make_async_copy(src, dst, in_sem.at[i])
             for i, (name, (src, dst)) in enumerate(pairs.items())}
    for c in loads.values():
        c.start()

    def wait(*names):
        for name in names:
            loads[name].wait()

    def store(j, rows):
        return pltpu.make_async_copy(out_s.at[rows], o_h.at[rows], out_sem.at[j])

    def clear(g, count):
        kprev_s[g] = jnp.zeros(kprev_s.shape[1:], i32)
        return count + 1

    tick = lax.fori_loop(0, NG, clear, 0)

    def ln1(i, r, n):
        x = x_s[pl.ds(_aligned(i * T1, T1) + r, n), :].astype(f32)
        xn_s[1, r:r + n, :] = _layernorm(x).astype(bf16)

    def qkv(i, first=False, last=False):
        tiles = range(T1 // QB)
        paced = () if last else (0,) if first else (0, 2)
        piece = T1 // (max(1, len(paced)) * len(tiles))
        done = [0]

        def proj_tile(j, b):
            y = _dot(xn_s[0, b * QB:(b + 1) * QB, :], wqkv_s[j])
            if j in paced:
                x_s[S:S + 8, 0:128] = y[0:8, 0:128].astype(bf16)
                ln1(i + 1 + tick // 4096, done[0], piece)
                done[0] += piece
            return y

        def put_v(b, y):
            vt_s[_W // QB + i * len(tiles) + b] = y.astype(bf16).astype(f32).T

        if first:
            wait("x0")
            ln1(0, 0, T1)
            wait("wv0")
            v0 = _dot(xn_s[1], wqkv_s[2, :, 0:_V_HEAD])
            wait("wv1")
            v1 = [_dot(xn_s[1, b * QB:(b + 1) * QB, :], wqkv_s[2, :, _V_HEAD:D]) for b in tiles]
            wait("wk")
            for b in tiles:
                put_v(b, jnp.concatenate([v0[b * QB:(b + 1) * QB], v1[b]], axis=1))
        k = jnp.concatenate(
            [pltpu.bitcast(_dot(xn_s[1, b * QB:(b + 1) * QB, :], wqkv_s[1]).astype(bf16), i32) for b in tiles],
            axis=0)
        xn_s[0] = xn_s[1]
        if first:
            wait("wq", "x1")
        lane = lax.broadcasted_iota(i32, (T1 // 2, 128), 1)
        rows = pl.ds(_aligned(_W // 2 - 32 + i * (T1 // 2), 32), T1 // 2)
        for g in range(NG):
            lo = 4 * Dh * g
            m = lo // 128
            kt = k[:, 128 * m:128 * (m + 1)]
            if (lo + 4 * Dh - 1) // 128 != m:
                kt = jnp.where(lane >= 64, kt, k[:, 128 * (m + 1):128 * (m + 2)])
            earlier = jnp.concatenate([kprev_s[g], kt[:T1 // 2 - 32]], axis=0)
            kprev_s[g] = kt[T1 // 2 - 32:]
            later = pltpu.roll(kt, 64, 1)
            for h0 in (4 * g, 4 * g + 2):
                even = jnp.where(((lane - Dh * h0) & 127) < 64, earlier, later)
                odd = pltpu.roll(even, 32, 1)
                for h in (h0, h0 + 1):
                    k_s[h, rows, :] = jnp.where(((lane - Dh * h) & 63) < 32, even, odd)
        yield True
        if not first:
            for b in tiles:
                put_v(b, proj_tile(2, b))
        yield True
        qscale = (Dh ** -0.5) * math.log2(math.e)
        for b in tiles:
            qt_s[i * len(tiles) + b] = pltpu.bitcast((proj_tile(0, b) * qscale).astype(bf16).T, i32)
        yield True

    recent = [None]

    def attention(blk, small):
        lane8 = lax.broadcasted_iota(i32, (8, QB), 1)
        row8 = lax.broadcasted_iota(i32, (8, QB), 0)
        diag8 = (lane8 & 63) - row8
        row16 = lax.broadcasted_iota(i32, (16, QB), 0)
        lane16 = lax.broadcasted_iota(i32, (16, QB), 1)
        head_rows = {o: jnp.where((row16 >= o) & (row16 < o + Dh // 2), -1, 0) for o in (0, 2, 4, 6)}
        slot_lanes = [jnp.where(lane16 // 32 == s, -1, 0) for s in range(4)]
        lane64 = lax.broadcasted_iota(i32, (64, QB), 1)
        left = lane64 < 64
        newest = lax.broadcasted_iota(i32, (64, QB), 0) <= (lane64 & 63)
        zw, zr = small // 4096, small // 8192
        s_s = (s0_s, s1_s)
        tile0 = blk * (T2 // QB)
        krow0 = _aligned(blk * (T2 // 2), T2 // 2)
        row_max = {}

        def gone(qb):
            return max(0, 4 - 2 * (tile0 + qb)) if isinstance(blk, int) else 0

        def live(qb, b):
            return b == 0 or b + 1 >= gone(qb)

        def scores(n, qb, g):
            qs = []
            for h in range(4 * g, 4 * g + 4):
                t0 = Dh * h // 16
                q = qt_s[tile0 + qb, 8 * t0:8 * t0 + 16, :]
                parts = [None] * 8
                for s in range(4):
                    qm = q & (head_rows[Dh * h // 2 - 8 * t0] & slot_lanes[s])
                    parts[(t0 + 2 * s) % 8], parts[(t0 + 2 * s + 1) % 8] = qm[0:8], qm[8:16]
                qs.append(pltpu.bitcast(jnp.concatenate(parts, axis=0), bf16))
            neg = jnp.full((8, QB), -jnp.inf, f32)
            mx = [None] * 4
            for chunk in _CHUNKS:
                chunk = [(b, r) for b, r in chunk if live(qb, b)]
                for u, h in enumerate(range(4 * g, 4 * g + 4)):
                    def keys(b, r):
                        return k_s[h, pl.ds(krow0 + (qb * QB + 64 * b + r) // 2, 8), :]

                    lhs = {}
                    for b, r in chunk:
                        if b:
                            lhs[b, r], lhs[b, r + 32] = keys(b, r), keys(b, r + 32)
                        elif gone(qb):
                            lhs[4, r], lhs["mix", r] = keys(4, r), keys(4, r + 32)
                        else:
                            lhs[4, r] = keys(4, r)
                            lhs["mix", r] = jnp.where(((lane8 - Dh * h) & 63) < 32, keys(0, r), keys(4, r + 32))
                            lhs[0, r + 32] = keys(0, r + 32)
                    st = _dot(pltpu.bitcast(jnp.concatenate(list(lhs.values()), axis=0), bf16), qs[u])
                    pos = {key: 16 * i for i, key in enumerate(lhs)}
                    for b, r in chunk:
                        for e in (0, 8):
                            def get(*key):
                                return st[pos[key] + e:pos[key] + e + 8] if key in pos else neg

                            if b == 0:
                                vals = (jnp.where(diag8 >= r + e, get(4, r), neg if gone(qb) else get("mix", r)),
                                        jnp.where(diag8 >= r + 32 + e, get("mix", r), get(0, r + 32)))
                            else:
                                vals = (get(b, r), get(b, r + 32))
                                if b < gone(qb):
                                    vals = tuple(jnp.where(lane8 < 64, neg, v) for v in vals)
                            for rr, v in zip((r, r + 32), vals):
                                s_s[n % 2][zw, pl.ds(64 * b + rr + e, 8), 128 * u:128 * (u + 1)] = v
                                mx[u] = v if mx[u] is None else jnp.maximum(mx[u], v)
                yield True
            row_max[n] = [jnp.max(m, axis=0, keepdims=True) for m in mx]

        def mix(n, qb, g):
            mx = row_max.pop(n)
            zero = jnp.zeros((64, QB), f32)

            @functools.cache
            def p(u, b):
                if not live(qb, b):
                    return zero
                return jnp.exp2(s_s[n % 2][zr, 64 * b:64 * (b + 1), 128 * u:128 * (u + 1)] - mx[u])

            def probs(u, t):
                if t == 0:
                    old = jnp.where(newest, zero, p(u, 0))
                    halves = [jnp.where(left, old, zero), jnp.where(left, p(u, 1), old)]
                elif t == 1:
                    halves = [jnp.where(left, p(u, 2), p(u, 1)), jnp.where(left, p(u, 3), p(u, 2))]
                else:
                    new = jnp.where(newest, p(u, 0), zero)
                    halves = [jnp.where(left, new, p(u, 3)), jnp.where(left, zero, new)]
                return jnp.concatenate(halves, axis=0)

            def values(h, t):
                a = Dh * h // 8 * 8
                vt = vt_s[tile0 + qb + t, a:a + 24, :]
                if h % 2:
                    return jnp.concatenate([jnp.where(row8 < 4, 1.0, vt[0:8]), vt[8:24]], axis=0)
                return jnp.concatenate([vt[0:16], jnp.where(row8 < 4, vt[16:24], 1.0)], axis=0)

            acc = [None] * 4
            for t in (0, 2, 1):
                for u in range(4 if 2 * t >= gone(qb) else 0):
                    o = _dot(values(4 * g + u, t), probs(u, t))
                    acc[u] = o if acc[u] is None else acc[u] + o
                if t != 1:
                    yield True
            recent[0] = acc[3][0:8]
            for u in (0, 2):
                a, b = acc[u] * (1.0 / acc[u][23:24]), acc[u + 1] * (1.0 / acc[u + 1][0:1])
                r = Dh * (4 * g + u)
                ot_s[qb, r:r + 2 * Dh, :] = jnp.concatenate(
                    [a[0:16], jnp.where(row8 < 4, a[16:24], b[0:8]), b[8:24]], axis=0)
            yield True

        units = [(qb, g) for qb in range(T2 // QB) for g in range(NG)]
        for n in range(len(units) + 1):
            stages = [scores(n, *units[n])] if n < len(units) else []
            stages += [mix(n - 1, *units[n - 1])] if n else []
            _interleave(stages)
            yield True

    def mlp(blk, last=False):
        row0 = _aligned(blk * T2, T2)
        whole = [slice(0, T2)]
        tiles = [slice(r, r + QB) for r in range(0, T2, QB)]

        def seq_rows(rs):
            return pl.ds(row0 + rs.start, rs.stop - rs.start)

        for b, rs in enumerate(tiles):
            att_s[rs, :] = ot_s[b].astype(bf16).T
        yield True
        for rs in tiles if last else whole:
            h_s[rs, :] = x_s[seq_rows(rs), :].astype(f32) + _dot(att_s[rs, :], wo_s[...])
            yield True
        n = QB if last else T2 // 4
        for r in range(0, T2, n):
            if last:
                h = h_s[r:r + n, :]
            else:
                h_s[T2:T2 + 8, 0:128] = recent[0]
                h = h_s[pl.ds(pl.multiple_of(r + blk // 4096 * 8, 8), n), :]
            hn_s[r:r + n, :] = _layernorm(h).astype(bf16)
            yield True
        b1 = b1_s[...].astype(f32).reshape(1, F)
        for c, e in ((0, _F_CUT), (_F_CUT, F)):
            for rs in tiles if last and c == 0 else whole:
                g_s[rs, c:e] = _gelu_x2(_dot(hn_s[rs, :], w1_s[:, c:e]) + b1[:, c:e]).astype(bf16)
                yield True
        b2 = b2_s[...].astype(f32).reshape(1, D)
        for j, rs in enumerate([slice(0, T2 - _LAST), slice(T2 - _LAST, T2)] if last else whole):
            y = _dot(g_s[rs, :], w2_s[...])
            out_s[seq_rows(rs), :] = (h_s[rs, :] + b2 + 0.5 * y).astype(out_s.dtype)
            store(blk + j, seq_rows(rs)).start()
            yield True

    def qkv_step(i, carry):
        _interleave([qkv(i)])
        return carry

    def block_step(i, carry):
        _trace_in_order(_ORDER, attention(i, i), mlp(i - 1))
        return carry

    _interleave([qkv(0, first=True)])
    wait("x2")
    lax.fori_loop(1, N1 - 1, qkv_step, 0)
    _trace_in_order("aafaaaaafaaaaaf", attention(0, tick), qkv(N1 - 1, last=True))
    wait("wo", "w1", "b1", "w2", "b2")
    lax.fori_loop(1, N2, block_step, 0)
    _interleave([mlp(N2 - 1, last=True)])
    for j in range(N2 - 1):
        store(j, pl.ds(j * T2, T2)).wait()
    store(N2 - 1, pl.ds(S - T2, T2 - _LAST)).wait()
    store(N2, pl.ds(S - _LAST, _LAST)).wait()


@jax.jit
def pallas_sequential_preLN__sliding_block__dense_activation_gelu__prompt_kernel(
    A_x: jax.Array,
    A_wqkv: jax.Array,
    A_wo: jax.Array,
    B_x: jax.Array,
    B_w1: jax.Array,
    B_b1: jax.Array,
    B_w2: jax.Array,
    B_b2: jax.Array,
):
    del B_x
    B, S, D = A_x.shape
    F = B_w1.shape[1]
    assert B == 1 and D == 20 * _H and S % _T1 == 0 and S >= 3 * _T1 and F > _F_CUT
    bf16, f32, i32 = jnp.bfloat16, jnp.float32, jnp.int32
    vmem = pltpu.VMEM
    out = pl.pallas_call(
        functools.partial(_kernel, S=S, D=D, F=F, Dh=D // _H),
        in_specs=[pl.BlockSpec(memory_space=pl.ANY)] * 7,
        out_specs=pl.BlockSpec(memory_space=pl.ANY),
        out_shape=jax.ShapeDtypeStruct((S, D), A_x.dtype),
        scratch_shapes=[
            vmem((S + 16, D), A_x.dtype),
            vmem((3, D, D), A_wqkv.dtype),
            vmem(A_wo.shape, A_wo.dtype),
            vmem(B_w1.shape, B_w1.dtype),
            vmem(B_b1.shape, B_b1.dtype),
            vmem(B_w2.shape, B_w2.dtype),
            vmem(B_b2.shape, B_b2.dtype),
            vmem((S, D), A_x.dtype),
            vmem((2, _T1, D), bf16),
            vmem((_H, (_W + S) // 2, 128), i32),
            vmem((_H // 4, 32, 128), i32),
            vmem(((_W + S) // _QB, D, _QB), f32),
            vmem((S // _QB, D // 2, _QB), i32),
            vmem((1, _W, 4 * _QB), f32),
            vmem((1, _W, 4 * _QB), f32),
            vmem((_T2 // _QB, D, _QB), f32),
            vmem((_T2, D), bf16),
            vmem((_T2 + 8, D), f32),
            vmem((_T2, D), bf16),
            vmem((_T2, F), bf16),
            pltpu.SemaphoreType.DMA((12,)),
            pltpu.SemaphoreType.DMA((S // _T2 + 1,)),
        ],
        compiler_params=pltpu.CompilerParams(vmem_limit_bytes=100 * 2**20),
    )(A_x.reshape(S, D), A_wqkv, A_wo, B_w1, B_b1, B_w2, B_b2)
    return out.reshape(B, S, D)
```
